```python
import os as _os
_os.environ.setdefault("JAX_PLATFORMS", "cpu")
import jax
import jax.numpy as jnp

def _softmax(x, axis=-1):
    return jax.nn.softmax(x, axis=axis)
def _gelu(x):
    return jax.nn.gelu(x, approximate=True)
def _silu(x):
    return jax.nn.silu(x)
def _sigmoid(x):
    return jax.nn.sigmoid(x)
def _layernorm(x, axis=-1, eps=1e-5):
    m = jnp.mean(x, axis=axis, keepdims=True)
    v = jnp.var(x, axis=axis, keepdims=True)
    return (x - m) / jnp.sqrt(v + eps)
def _scatter_add(tgt, idx, src, axis=0):
    return tgt.at[idx].add(src)
def _segment_sum(src, seg, n):
    return jax.ops.segment_sum(src, seg, n)
class _Rng:
    def __init__(self, key):
        self._k = key
    def _next(self):
        self._k, sub = jax.random.split(self._k)
        return sub
    def normal(self, shape):
        return jax.random.normal(self._next(), shape, dtype=jnp.bfloat16)
    def randint(self, lo, hi, shape):
        return jax.random.randint(self._next(), shape, lo, hi, dtype=jnp.int32)
    def uniform(self, shape, lo=0.0, hi=1.0):
        return jax.random.uniform(self._next(), shape, jnp.bfloat16, lo, hi)
    def permutation(self, n):
        return jax.random.permutation(self._next(), n)


kernel_name = 'parallel_sum__grouped_kv_mqa__dense_activation_silu__prompt'

def setup_inputs():
    _rng = _Rng(jax.random.key(int.from_bytes(__import__("os").urandom(4), "little")))
    _w = (lambda a: (lambda t: t.astype(jnp.bfloat16) if jnp.issubdtype(t.dtype, jnp.floating) else t)(jnp.asarray(a)))
    def _A_setup():
        B, S, D, H = 1, 2048, 512, 32
        Dh = D // H
        return {
            "x": _w((lambda *s: _rng.normal(s) * 0.05)(B, S, D)),
            "wq": _w((lambda *s: _rng.normal(s) * 0.05)(D, H * Dh)),
            "wk": _w((lambda *s: _rng.normal(s) * 0.05)(D, Dh)),
            "wv": _w((lambda *s: _rng.normal(s) * 0.05)(D, Dh)),
            "wo": _w((lambda *s: _rng.normal(s) * 0.05)(H * Dh, D)),
        }
    _A_in = _A_setup()

    def _B_setup():
        B, S, D, F = 1, 2048, 512, 1792
        return {
            "x": _w((lambda *s: _rng.normal(s) * 0.05)(B, S, D)),
            "w1": _w((lambda *s: _rng.normal(s) * 0.05)(D, F) * (D ** -0.5)),
            "w2": _w((lambda *s: _rng.normal(s) * 0.05)(F, D) * (F ** -0.5)),
        }
    _B_in = _B_setup()

    return {
        "A_x": _A_in["x"],
        "A_wq": _A_in["wq"],
        "A_wk": _A_in["wk"],
        "A_wv": _A_in["wv"],
        "A_wo": _A_in["wo"],
        "B_x": _B_in["x"],
        "B_w1": _B_in["w1"],
        "B_w2": _B_in["w2"],
    }

def reference(A_x, A_wq, A_wk, A_wv, A_wo, B_x, B_w1, B_w2):
    def _A_ref(x, wq, wk, wv, wo):
        B, S, D = x.shape
        H = 32
        Dh = D // H
        q = (lambda x, *d: x.transpose(*d))((x @ wq).reshape(B, S, H, Dh), 0, 2, 1, 3)
        k = x @ wk
        v = x @ wv
        scores = jnp.einsum("bhqd,bkd->bhqk", q, k) * (Dh ** -0.5)
        p = _softmax(scores, axis=-1)
        o = jnp.einsum("bhqk,bkd->bhqd", p, v)
        return (lambda x, *d: x.transpose(*d))(o, 0, 2, 1, 3).reshape(B, S, H * Dh) @ wo

    def _B_ref(x, w1, w2):
        h = jnp.einsum("bsd,df->bsf", x, w1)
        h = _silu(h)
        out = jnp.einsum("bsf,fd->bsd", h, w2)
        return out

    x = A_x
    xn = _layernorm(x, axis=-1)
    return x + _A_ref(xn, A_wq, A_wk, A_wv, A_wo) + _B_ref(xn, B_w1, B_w2)
```

```python
import math

import jax
import jax.numpy as jnp
import jax.experimental.pallas as pl
import jax.experimental.pallas.tpu as pltpu

F32 = jnp.float32
BF16 = jnp.bfloat16
U32 = jnp.uint32

S = 2048
D = 512
H = 32
DH = 16
FF = 1792
TQ = 512
NQ = S // TQ
EPS = 1e-5
QSCALE = (DH ** -0.5) * math.log2(math.e)
KC = 128
LN_ROWS = 256
FC = 256
L_SAFE = 2.0 ** -60


def _pk(x):
    return pltpu.bitcast(x, U32)


def _upk(x):
    return pltpu.bitcast(x, BF16)


def _kernel(x_ref, wq_ref, wk_ref, wv_ref, wo_ref, w1_ref, w2_ref, o_ref,
            xn_scr, wqt_scr, k_scr, vt_scr, kmax_scr, qt_scr, p_scr, l_scr, lmin_scr, ot_scr):
    i = pl.program_id(0)

    @pl.when(i == 0)
    def _():
        wqt_scr[...] = _pk(wq_ref[...].astype(F32).T.astype(BF16))
        wkv = jnp.concatenate(
            [wk_ref[...].astype(F32), wv_ref[...].astype(F32), jnp.zeros((D, 128 - 2 * DH), F32)], axis=1
        ).astype(BF16)
        lane = jax.lax.broadcasted_iota(jnp.int32, (LN_ROWS, 128), 1)
        kmax_scr[...] = jnp.zeros((8, 128), F32)

        def ln_chunk(c, carry):
            r0 = pl.multiple_of(c * LN_ROWS, LN_ROWS)
            x = x_ref[0, pl.ds(r0, LN_ROWS), :].astype(F32)
            mu = jnp.mean(x, axis=-1, keepdims=True)
            xc = x - mu
            var = jnp.mean(xc * xc, axis=-1, keepdims=True)
            xn = (xc * jax.lax.rsqrt(var + EPS)).astype(BF16)
            xn_scr[pl.ds(pl.multiple_of(c * (LN_ROWS // 2), LN_ROWS // 2), LN_ROWS // 2), :] = _pk(xn)
            kv = jnp.dot(xn, wkv, preferred_element_type=F32).astype(BF16).astype(F32)
            kvt = kv.T
            vt_scr[:, pl.ds(r0, LN_ROWS)] = _pk(kvt[DH:2 * DH, :].astype(BF16))
            kt = kvt[0:DH, :]
            k2 = jnp.sum(kt * kt, axis=0, keepdims=True)
            k2m = jnp.max(k2, axis=1, keepdims=True)
            kmax_scr[...] = jnp.maximum(kmax_scr[...], jnp.broadcast_to(k2m, (8, 128)))
            kaug = jnp.where(lane < DH, kv, jnp.where(lane == DH, 1.0, 0.0))
            kp = _pk(kaug.astype(BF16))
            ev = pltpu.unpack_elementwise(kp, index=0, packed_dtype=BF16, unpacked_dtype=F32)
            od = pltpu.unpack_elementwise(kp, index=1, packed_dtype=BF16, unpacked_dtype=F32)
            kperm = jnp.concatenate(
                [ev.reshape(LN_ROWS // 16, 1, 8, 128), od.reshape(LN_ROWS // 16, 1, 8, 128)], axis=1
            ).reshape(LN_ROWS, 128)
            k_scr[pl.ds(pl.multiple_of(c * (LN_ROWS // 2), LN_ROWS // 2), LN_ROWS // 2), :] = _pk(kperm.astype(BF16))
            return carry

        jax.lax.fori_loop(0, S // LN_ROWS, ln_chunk, 0)

    xn_rows = pl.ds(pl.multiple_of(i * (TQ // 2), TQ // 2), TQ // 2)
    xn_t = _upk(xn_scr[xn_rows, :])
    qt = jax.lax.dot_general(_upk(wqt_scr[...]), xn_t, (((1,), (1,)), ((), ())),
                             preferred_element_type=F32)
    qt = (qt * QSCALE).astype(BF16).astype(F32).reshape(H, DH, TQ)
    q2 = jnp.sum(qt * qt, axis=1, keepdims=True)
    kmax2 = kmax_scr[0:1, 0:1].reshape(1, 1, 1)
    mb = jnp.sqrt(q2 * kmax2) * (1.0 + 2.0 ** -6)
    row = jax.lax.broadcasted_iota(jnp.int32, (H, DH, TQ), 1)
    mrow = jnp.where(row == 0, -mb, 0.0)
    qaug = jnp.concatenate([qt, mrow], axis=1).reshape(H * 2 * DH, TQ).astype(BF16)
    qt_scr[...] = _pk(qaug).reshape(H, DH, TQ)

    def store_p(p, r0, nr, slot):
        p4 = p.reshape(nr // 16, 2, 8, TQ)
        pp = pltpu.pack_elementwise([p4[:, 0], p4[:, 1]], packed_dtype=BF16)
        p_scr[slot, r0 // 2:(r0 + nr) // 2, :] = pp.reshape(nr // 2, TQ).astype(U32)
        return jnp.sum(p.reshape(nr // 8, 8, TQ), axis=0)

    def qk_piece(h, c, slot, l):
        kk = _upk(k_scr[c * KC // 2:(c + 1) * KC // 2, :])[:, :2 * DH]
        s = jnp.dot(kk, _upk(qt_scr[h]), preferred_element_type=F32)
        return l + store_p(jnp.exp2(s), c * KC, KC, slot)

    def pv_tile(t, slot, acc):
        return acc + jnp.dot(_upk(vt_scr[:, t * 128:(t + 1) * 128]),
                             _upk(p_scr[slot, t * 64:(t + 1) * 64, :]),
                             preferred_element_type=F32)

    def finish(h, acc, l):
        lsum = jnp.sum(l, axis=0, keepdims=True)
        ot_scr[h] = acc / lsum
        return lsum

    def unit(hq, slot, hpv):
        l = jnp.zeros((8, TQ), F32)
        acc = jnp.zeros((DH, TQ), F32)
        if hpv is not None:
            lprev = l_scr[...]
        for c in range(S // KC):
            if hq is not None:
                l = qk_piece(hq, c, slot, l)
            if hpv is not None:
                for t in range(c * KC // 128, (c + 1) * KC // 128):
                    acc = pv_tile(t, 1 - slot, acc)
        if hpv is not None:
            lsum = finish(hpv, acc, lprev)
            lmin_scr[...] = jnp.minimum(lmin_scr[...], lsum)
        if hq is not None:
            l_scr[...] = l

    lmin_scr[...] = jnp.full((1, TQ), jnp.inf, F32)
    unit(0, 0, None)

    def body(hh, carry):
        h = 2 * hh + 1
        unit(h, 1, h - 1)
        unit(h + 1, 0, h)
        return carry

    jax.lax.fori_loop(0, H // 2 - 1, body, 0)
    unit(H - 1, 1, H - 2)
    unit(None, 0, H - 1)

    safe = jnp.min(lmin_scr[...]) >= L_SAFE

    @pl.when(jnp.logical_not(safe))
    def _():
        def slow_head(h, carry):
            kk = _upk(k_scr[...])[:, :DH]
            s = jnp.dot(kk, _upk(qt_scr[h, 0:DH // 2, :]), preferred_element_type=F32)
            m = jnp.max(s, axis=0, keepdims=True)
            l = store_p(jnp.exp2(s - m), 0, S, 0)
            acc = jnp.dot(_upk(vt_scr[...]), _upk(p_scr[0]), preferred_element_type=F32)
            finish(h, acc, l)
            return carry

        jax.lax.fori_loop(0, H, slow_head, 0)

    o = ot_scr[...].reshape(D, TQ).T.astype(BF16)
    acc = jnp.dot(o, wo_ref[...], preferred_element_type=F32)
    acc = acc + x_ref[0, pl.ds(pl.multiple_of(i * TQ, TQ), TQ), :].astype(F32)
    for f in range(FF // FC):
        hcol = jnp.dot(xn_t, w1_ref[:, f * FC:(f + 1) * FC], preferred_element_type=F32)
        u = 0.5 * hcol
        hact = (u * jnp.tanh(u) + u).astype(BF16)
        acc = acc + jnp.dot(hact, w2_ref[f * FC:(f + 1) * FC, :], preferred_element_type=F32)
    o_ref[0] = acc.astype(BF16)


@jax.jit
def pallas_parallel_sum__grouped_kv_mqa__dense_activation_silu__prompt_kernel(
    A_x: jax.Array,
    A_wq: jax.Array,
    A_wk: jax.Array,
    A_wv: jax.Array,
    A_wo: jax.Array,
    B_x: jax.Array,
    B_w1: jax.Array,
    B_w2: jax.Array,
):
    del B_x
    full = lambda shape: pl.BlockSpec(shape, lambda i: (0,) * len(shape))
    return pl.pallas_call(
        _kernel,
        out_shape=jax.ShapeDtypeStruct((1, S, D), BF16),
        grid=(NQ,),
        in_specs=[
            full((1, S, D)), full((D, D)), full((D, DH)), full((D, DH)), full((D, D)),
            full((D, FF)), full((FF, D)),
        ],
        out_specs=pl.BlockSpec((1, TQ, D), lambda i: (0, i, 0)),
        scratch_shapes=[
            pltpu.VMEM((S // 2, D), U32),
            pltpu.VMEM((D // 2, D), U32),
            pltpu.VMEM((S // 2, 128), U32),
            pltpu.VMEM((DH // 2, S), U32),
            pltpu.VMEM((8, 128), F32),
            pltpu.VMEM((H, DH, TQ), U32),
            pltpu.VMEM((2, S // 2, TQ), U32),
            pltpu.VMEM((8, TQ), F32),
            pltpu.VMEM((1, TQ), F32),
            pltpu.VMEM((H, DH, TQ), F32),
        ],
        compiler_params=pltpu.CompilerParams(
            dimension_semantics=("arbitrary",),
            vmem_limit_bytes=100 * 1024 * 1024,
        ),
    )(A_x, A_wq, A_wk, A_wv, A_wo, B_w1, B_w2)
```

```python
import math

import jax
import jax.numpy as jnp
import jax.experimental.pallas as pl
import jax.experimental.pallas.tpu as pltpu

F32 = jnp.float32
BF16 = jnp.bfloat16
U32 = jnp.uint32

S = 2048
D = 512
H = 32
DH = 16
FF = 1792
TQ = 512
NL = TQ // 128
NQ = S // TQ
EPS = 1e-5
QSCALE = (DH ** -0.5) * math.log2(math.e)
CH = 256
NCH = S // CH
NP = 4
HP = H // NP
FC = 256
L_SAFE = 2.0 ** -60
UP = 1.0 + 2.0 ** -7

import os, json
_C = json.loads(os.environ.get("KCFG", "{}"))
RVS = _C.get("RVS", [288, 288])
UPI = len(RVS)
RV = max(RVS)
W = _C.get("W", 3)
ND = _C.get("ND", 16)
FIRST = _C.get("FIRST", 6)
RELG = _C.get("RELG", 14)
TAIL = _C.get("TAIL", 0)
GLOBAL = _C.get("GLOBAL", 0)
NS = RV // (16 * W)
NT = S // 128
KB0 = -(-RV // CH)
TINY = 1e-30
XWAIT = {int(k): v for k, v in _C.get('XWAIT', {'1': [2, 3, 4], '4': [5, 6, 7]}).items()}


RVF = _C.get("RVF", [336, 336])
FR = _C.get("FR", 256)
RELT = _C.get("RELT", [256, 256])
FT0 = _C.get("FT0", [96, 64])
RV = max(RVS + RVF)
NS = RV // (16 * W)
KB0 = -(-RV // CH)
NFC = FF // 128


class _Plan:
    def __init__(self, rv, first, ffn=None, prev=None):
        self.g0 = rv // 16
        self.g = (S - rv) // 16
        self.bounds = [self.g * c // ND for c in range(ND + 1)]
        self.vsteps = [(j, t) for j in range(NL) for t in range(rv // (16 * W))]
        nv = len(self.vsteps)
        nvt = -(-rv // 128)
        self.pv_order = list(range(nvt, NT)) + list(range(nvt))
        self.ffn = ffn
        if ffn is None:
            self.fpos = {}
            self.dl = [first + (self.g - 1 - first) * v // (nv - 1) for v in range(nv)]
            self.rel = [d - RELG if d >= RELG else ("p", self.g + d - RELG) for d in self.dl]
            self.order = {g: 2 * c for c in range(ND) for g in range(self.bounds[c], self.bounds[c + 1])}
        else:
            npc = TQ // FR
            self.fpos = {(2 * p + 1) * ND // (2 * npc): p for p in range(npc)}
            t = 0
            self.t = {}
            self.order = {}
            for c in range(ND):
                for g in range(self.bounds[c], self.bounds[c + 1]):
                    self.t[g] = t
                    self.order[g] = 2 * c
                    t += 16
                t += 16 * NT // ND
                if c in self.fpos:
                    for gi in range(FR // 16):
                        self.t[("f", self.fpos[c], gi)] = t
                        self.order[("f", self.fpos[c], gi)] = 2 * c + 1
                        t += 16
            self.total = t
            tl = dict(self.t)
            if prev is not None:
                tl.update({("p", g): tt - prev.total for g, tt in prev.t.items()})
            tend = max(self.t.values()) - _C.get('TEND', [0, 0])[ffn - 1]
            self.dl, self.rel = [], []
            for v in range(nv):
                want = first + (tend - first) * v // (nv - 1)
                d = min((g for g in self.t if self.t[g] >= want), key=self.t.get)
                self.dl.append(d)
                cand = [g for g in tl if tl[g] <= self.t[d] - RELT[ffn - 1]]
                self.rel.append(max(cand, key=tl.get) if cand else None)


F2 = _C.get("F2", 3)
PLANS = [_Plan(rv, FIRST if u == 0 else F2) for u, rv in enumerate(RVS)]
_pa = _Plan(RVF[0], FT0[0], ffn=1)
FPLANS = [_pa, _Plan(RVF[1], FT0[1], ffn=2, prev=_pa)]

NT_DIMS = (((1,), (1,)), ((), ()))


def _pk(x):
    return pltpu.bitcast(x, U32)


def _upk(x):
    return pltpu.bitcast(x, BF16)


def _layernorm(x):
    x = x.astype(F32)
    mu = jnp.mean(x, axis=-1, keepdims=True)
    xc = x - mu
    var = jnp.mean(xc * xc, axis=-1, keepdims=True)
    return (xc * jax.lax.rsqrt(var + EPS)).astype(BF16)


def _kernel(x_hbm, wq_hbm, wkt_hbm, wvt_hbm, wo_hbm, w1_hbm, w2_hbm, o_ref,
            x_scr, wq_scr, wkt_ref, wvt_ref, wo_scr, w1_scr, w2_scr, sems,
            xn_scr, wt_scr, k_scr, vt_scr, kmax_scr, qt_scr, p_scr, l_scr, lmin_scr, ot_scr,
            z_scr, kvo_scr, kb_scr, qc_scr, qtc_scr, h_scr, acc_scr, bak_scr):
    i = pl.program_id(0)

    def x_copy(c):
        rows = pl.ds(c * CH, CH)
        return pltpu.make_async_copy(x_hbm.at[0, rows, :], x_scr.at[rows, :], sems.at[c])

    wq_copy = pltpu.make_async_copy(wq_hbm, wq_scr, sems.at[NCH])
    kv_copies = [pltpu.make_async_copy(wkt_hbm, wkt_ref, sems.at[NCH + 4]),
                 pltpu.make_async_copy(wvt_hbm, wvt_ref, sems.at[NCH + 5])]
    w_copies = [pltpu.make_async_copy(w1_hbm, w1_scr, sems.at[NCH + 1]),
                pltpu.make_async_copy(w2_hbm, w2_scr, sems.at[NCH + 2]),
                pltpu.make_async_copy(wo_hbm, wo_scr, sems.at[NCH + 3])]

    def tie(x, dep):
        r = pltpu.bitcast(dep, U32) & z_scr[...]
        if x.shape[0] != 8:
            r = jnp.concatenate([r] * (x.shape[0] // 8), axis=0)
        return pltpu.bitcast(pltpu.bitcast(x, U32) | r, x.dtype)

    def store_p(p, r0, nr, slot):
        p4 = p.reshape(nr // 16, 2, 8, TQ)
        pp = pltpu.pack_elementwise([p4[:, 0], p4[:, 1]], packed_dtype=BF16)
        p_scr[slot, r0 // 2:(r0 + nr) // 2, :] = pp.reshape(nr // 2, TQ).astype(U32)
        return jnp.sum(p.reshape(nr // 8, 8, TQ), axis=0)

    def qk_dot(pn, c, slot, l, deps, rels):
        g0, g1 = pn.bounds[c], pn.bounds[c + 1]
        G0 = pn.g0
        ks = []
        for g in range(g0, g1):
            kv = k_scr[(G0 + g) * 8:(G0 + g + 1) * 8, :]
            if g in deps:
                kv = tie(kv, deps[g])
            ks.append(kv)
        kk = _upk(jnp.concatenate(ks, axis=0))[:, :2 * DH]
        s = jnp.dot(kk, _upk(qtc_scr[slot]), preferred_element_type=F32)
        for g in range(g0, g1):
            rels[g] = s[(g - g0) * 16:(g - g0) * 16 + 8, 0:128]
        return l + store_p(jnp.exp2(s), (G0 + g0) * 16, (g1 - g0) * 16, slot)

    def vpu_step(pn, v, slot, lv, acc, rel):
        j, t = pn.vsteps[v]
        c0 = j * 128
        if t == 0:
            m8 = jnp.broadcast_to(qc_scr[slot, DH:DH + 1, c0:c0 + 128], (8, 128)) * kmax_scr[...]
            if rel is not None:
                m8 = tie(m8, rel)
            mm = jnp.concatenate([m8] * W, axis=0)
            if acc is not None:
                zz = jnp.concatenate([z_scr[...]] * W, axis=0)
                mm = pltpu.bitcast(pltpu.bitcast(mm, U32) | (pltpu.bitcast(acc, U32) & zz), F32)
            acc = mm
        elif rel is not None:
            acc = tie(acc, rel)
        ps = []
        for b in range(2):
            r0 = (2 * t + b) * 8 * W
            for d in range(DH):
                acc = acc + kb_scr[0, d, r0:r0 + 8 * W, :] * qc_scr[slot, d:d + 1, c0:c0 + 128]
            ps.append(jnp.exp2(acc))
        pp = pltpu.pack_elementwise(ps, packed_dtype=BF16)
        pr0 = t * 8 * W
        p_scr[slot, pr0:pr0 + 8 * W, c0:c0 + 128] = pp.astype(U32)
        lv = list(lv)
        lv[j] = lv[j] + jnp.sum((ps[0] + ps[1]).reshape(W, 8, 128), axis=0)
        return lv, acc

    def pv_tile(t, slot, acc):
        return acc + jnp.dot(_upk(vt_scr[:, t * 128:(t + 1) * 128]),
                             _upk(p_scr[slot, t * 64:(t + 1) * 64, :]),
                             preferred_element_type=F32)

    def finish(h, acc, l):
        lsum = jnp.sum(l, axis=0, keepdims=True)
        ot_scr[h] = acc / lsum
        return lsum

    def stage_q(n, slot):
        q = qt_scr[n]
        qtc_scr[slot] = q
        qc_scr[slot] = _upk(q).astype(F32)[:DH + 8]

    def stage_tile(t):
        acc_scr[...] = x_scr[pl.ds(pl.multiple_of(t * TQ, TQ), TQ), :].astype(F32)

    def ffn_piece(kind, p, f, deps, rels):
        rows = pl.ds(p * FR, FR)
        if kind == 1:
            wrap = f + 1 >= NFC
            f = jnp.where(wrap, 0, f + 1)
            t = jnp.where(wrap, jnp.minimum(i + 1, NQ - 1), i)
            lhs = xn_scr[pl.ds(pl.multiple_of(t * (TQ // 2) + p * (FR // 2), FR // 2), FR // 2), :]
        else:
            lhs = _pk(h_scr[rows, :])
        fcols = pl.ds(pl.multiple_of(f * 128, 128), 128)
        gs = []
        for gi in range(FR // 16):
            g = lhs[gi * 8:(gi + 1) * 8]
            if ("f", p, gi) in deps:
                g0 = tie(g[:, :128], deps[("f", p, gi)])
                g = g0 if kind == 2 else jnp.concatenate([g0, g[:, 128:]], axis=1)
            gs.append(g)
        lhs = _upk(jnp.concatenate(gs, axis=0))
        r = jnp.dot(lhs, w1_scr[:, fcols] if kind == 1 else w2_scr[fcols, :], preferred_element_type=F32)
        for gi in range(FR // 16):
            rels[("f", p, gi)] = r[gi * 16:gi * 16 + 8, :128]
        if kind == 1:
            u = 0.5 * r
            h_scr[rows, :] = (u * jnp.tanh(u) + u).astype(BF16)
        else:
            acc_scr[rows, :] += r

    def unit(pn, pprev, slot, hpv, vacc=None, crel=None, f=None):
        l = jnp.zeros((8, TQ), F32)
        lv = [jnp.zeros((8, 128), F32) for _ in range(NL)]
        acc = jnp.zeros((DH, TQ), F32)
        if hpv is not None:
            lprev = l_scr[...]
        vb = 0
        tb = 0
        deps = {}
        rels = dict(crel or {})
        nv = len(pn.vsteps)
        for m in range(2 * ND):
            c = m // 2
            while vb < nv and pn.order[pn.dl[vb]] <= m:
                lv, vacc = vpu_step(pn, vb, slot, lv, vacc, rels.get(pn.rel[vb]))
                assert pn.dl[vb] not in deps
                deps[pn.dl[vb]] = lv[pn.vsteps[vb][0]]
                vb += 1
            if m % 2 == 0:
                l = qk_dot(pn, c, slot, l, deps, rels)
                while hpv is not None and tb < (c + 1) * NT // ND:
                    acc = pv_tile(pprev.pv_order[tb], 1 - slot, acc)
                    tb += 1
            elif c in pn.fpos:
                ffn_piece(3 - pn.ffn, pn.fpos[c], f, deps, rels)
        if hpv is not None:
            lsum = finish(hpv, acc, lprev)
            lmin_scr[...] = jnp.minimum(lmin_scr[...], lsum)
        l_scr[...] = l + jnp.concatenate(lv, axis=1)
        return vacc, {("p", g): r for g, r in rels.items()}

    def split_pairs(k):
        n = k.shape[0]
        kp = _pk(k.astype(BF16))
        ev = pltpu.unpack_elementwise(kp, index=0, packed_dtype=BF16, unpacked_dtype=F32)
        od = pltpu.unpack_elementwise(kp, index=1, packed_dtype=BF16, unpacked_dtype=F32)
        return ev.reshape(n // 16, 8, 128), od.reshape(n // 16, 8, 128)

    @pl.when(i == 0)
    def _():
        x_copy(0).start()
        for cp in kv_copies:
            cp.start()
        wq_copy.start()
        for c in range(1, NCH):
            x_copy(c).start()
        z_scr[...] = jnp.zeros((8, 128), U32)
        x_copy(0).wait()
        xn_scr[0:CH // 2, :] = _pk(_layernorm(x_scr[0:CH, :]))
        for cp in kv_copies:
            cp.wait()
        wq_copy.wait()
        x_copy(1).wait()
        wkv = jnp.concatenate([wkt_ref[...].astype(F32), wvt_ref[...].astype(F32)], axis=0)
        wt_scr[:DH, :] = _pk(wkv.astype(BF16))
        wt_scr[DH:, :] = _pk(wq_scr[...].astype(F32).T.astype(BF16))

        row = jax.lax.broadcasted_iota(jnp.int32, (HP, DH, CH), 1)
        kmax2 = jnp.zeros((1, CH), F32)
        evs, ods = [], []
        nslots = (NCH - KB0) * NP
        for c in range(NCH if not _C.get('FAST') else 0):
            if c in XWAIT:
                for cw in XWAIT[c]:
                    x_copy(cw).wait()
                if max(XWAIT[c]) == NCH - 1:
                    for cp in w_copies:
                        cp.start()
            half = pl.ds(c * (CH // 2), CH // 2)
            xn = _upk(xn_scr[half, :])
            if c < NCH - 1:
                xn_scr[(c + 1) * (CH // 2):(c + 2) * (CH // 2), :] = _pk(
                    _layernorm(x_scr[(c + 1) * CH:(c + 2) * CH, :]))
            tile = c // (TQ // CH)
            cols = pl.ds((c % (TQ // CH)) * CH, CH)
            for pc in range(NP):
                r1 = 2 * DH + (pc + 1) * HP * DH
                r0 = 0 if pc == 0 else r1 - HP * DH
                t_all = jax.lax.dot_general(_upk(wt_scr[r0 // 2:r1 // 2, :]), xn, NT_DIMS,
                                            preferred_element_type=F32)
                if pc == 0:
                    vt_scr[:, pl.ds(c * CH, CH)] = _pk(t_all[DH:2 * DH].astype(BF16))
                    kt = t_all[:DH].astype(BF16).astype(F32)
                    kmax2 = jnp.maximum(kmax2, jnp.sum(kt * kt, axis=0, keepdims=True))
                    k = jnp.concatenate([kt, jnp.zeros((128 - DH, CH), F32)], axis=0).T
                    ev, od = split_pairs(k)
                    kperm = jnp.concatenate([ev[:, None], od[:, None]], axis=1).reshape(CH, 128)
                    k_scr[half, :] = _pk(kperm.astype(BF16))
                    if c < KB0:
                        evs.append(ev)
                        ods.append(od)
                    if c == KB0 - 1:
                        ev = jnp.concatenate(evs, axis=0)
                        od = jnp.concatenate(ods, axis=0)
                        parts = []
                        for t in range(NS):
                            parts.append(ev[W * t:W * (t + 1)].reshape(8 * W, 128))
                            parts.append(od[W * t:W * (t + 1)].reshape(8 * W, 128))
                        kvo = jnp.concatenate(parts, axis=0)
                        kvo_scr[...] = jnp.concatenate(
                            [kvo[:8 * W], kvo[8 * W:] - kvo[:RV - 8 * W]], axis=0)
                    t_all = t_all[2 * DH:]
                qt = (t_all * QSCALE).astype(BF16).astype(F32).reshape(HP, DH, CH)
                q2 = jnp.sum(qt * qt, axis=1, keepdims=True) + TINY
                qn = q2 * jax.lax.rsqrt(q2) * (-UP)
                qaug = jnp.concatenate([qt, jnp.where(row == 0, qn, 0.0)], axis=1)
                qp = _pk(qaug.reshape(HP * 2 * DH, CH).astype(BF16)).reshape(HP, DH, CH)
                qt_scr[pl.ds(tile * H + pc * HP, HP), :, cols] = qp
                if c >= KB0:
                    sl = (c - KB0) * NP + pc
                    for d in range(DH * sl // nslots, DH * (sl + 1) // nslots):
                        src = tie(kvo_scr[...], t_all[0:8, 0:128])
                        kb_scr[0, d] = jnp.broadcast_to(src[:, d:d + 1], (RV, 128))

        kmax_scr[...] = jnp.broadcast_to(jnp.max(kmax2, axis=1, keepdims=True), (8, 128))
        km = (jnp.sqrt(kmax_scr[...]) * UP).astype(BF16).astype(F32)
        kmax_scr[...] = km
        kmw = pltpu.pack_elementwise([km, km], packed_dtype=BF16).astype(U32)
        lane = jax.lax.broadcasted_iota(jnp.int32, (S // 16, 8, 128), 2)
        k_scr[...] = jnp.where(lane == DH, kmw[None], k_scr[...].reshape(S // 16, 8, 128)).reshape(S // 2, 128)
        stage_tile(0)
        stage_q(0, 0)
        stage_q(1, 1)
        if not _C.get('FAST'):
            unit(PLANS[-1], None, 0, None)
        stage_q(2, 0)

    lmin_scr[...] = jnp.full((1, TQ), jnp.inf, F32)
    n0 = i * H
    last = NQ * H - 1

    def make_body(plans, h0):
        def body(hh, carry):
            va, cr = None, None
            for u in range(UPI):
                h = h0 + UPI * hh + u
                va, cr = unit(plans[u], plans[u - 1], (u + 1) % 2, h, va, cr, hh)
                stage_q(jnp.minimum(n0 + h + 3, last), (u + 1) % 2)
            return carry
        return body

    if _C.get('FAST', 0) != 1:
        jax.lax.fori_loop(0, H // UPI - NFC, make_body(PLANS, 0), 0)

    @pl.when(i == 0)
    def _():
        for cp in w_copies:
            cp.wait()
        for p in range(TQ // FR):
            ffn_piece(1, p, -1, {}, {})

    is_last = i == NQ - 1
    if _C.get('FAST', 0) != 2:
        jax.lax.fori_loop(0, NFC - is_last.astype(jnp.int32), make_body(FPLANS, H - UPI * NFC), 0)

    @pl.when(is_last)
    def _():
        if not _C.get('FAST'):
            unit(FPLANS[0], FPLANS[1], 1, H - 2, f=NFC - 1)
            acc = jnp.zeros((DH, TQ), F32)
            for t in FPLANS[0].pv_order:
                acc = pv_tile(t, 1, acc)
            lmin_scr[...] = jnp.minimum(lmin_scr[...], finish(H - 1, acc, l_scr[...]))

    def out_proj(base):
        o = ot_scr[...].reshape(D, TQ).T.astype(BF16)
        o_ref[0] = (jnp.dot(o, wo_scr[...], preferred_element_type=F32) + base).astype(BF16)

    safe = jnp.min(lmin_scr[...]) >= L_SAFE
    base = acc_scr[...]
    bak_scr[...] = base
    out_proj(base)
    stage_tile(jnp.minimum(i + 1, NQ - 1))

    @pl.when(jnp.logical_not(safe))
    def _():
        def slow_head(h, carry):
            kk = _upk(k_scr[...])[:, :DH]
            s = jnp.dot(kk, _upk(qt_scr[n0 + h, 0:DH // 2, :]), preferred_element_type=F32)
            m = jnp.max(s, axis=0, keepdims=True)
            l = store_p(jnp.exp2(s - m), 0, S, 1)
            acc = jnp.dot(_upk(vt_scr[...]), _upk(p_scr[1]), preferred_element_type=F32)
            finish(h, acc, l)
            return carry

        if not _C.get('FAST'):
            jax.lax.fori_loop(0, H, slow_head, 0)
            out_proj(bak_scr[...])


@jax.jit
def pallas_parallel_sum__grouped_kv_mqa__dense_activation_silu__prompt_kernel(
    A_x: jax.Array,
    A_wq: jax.Array,
    A_wk: jax.Array,
    A_wv: jax.Array,
    A_wo: jax.Array,
    B_x: jax.Array,
    B_w1: jax.Array,
    B_w2: jax.Array,
):
    del B_x
    hbm = pl.BlockSpec(memory_space=pl.ANY)
    return pl.pallas_call(
        _kernel,
        out_shape=jax.ShapeDtypeStruct((1, S, D), BF16),
        grid=(NQ,),
        in_specs=[hbm] * 7,
        out_specs=pl.BlockSpec((1, TQ, D), lambda i: (0, i, 0)),
        scratch_shapes=[
            pltpu.VMEM((S, D), BF16),
            pltpu.VMEM((D, D), BF16),
            pltpu.VMEM((DH, D), BF16),
            pltpu.VMEM((DH, D), BF16),
            pltpu.VMEM((D, D), BF16),
            pltpu.VMEM((D, FF), BF16),
            pltpu.VMEM((FF, D), BF16),
            pltpu.SemaphoreType.DMA((NCH + 6,)),
            pltpu.VMEM((S // 2, D), U32),
            pltpu.VMEM((D // 2 + DH, D), U32),
            pltpu.VMEM((S // 2, 128), U32),
            pltpu.VMEM((DH // 2, S), U32),
            pltpu.VMEM((8, 128), F32),
            pltpu.VMEM((NQ * H, DH, TQ), U32),
            pltpu.VMEM((2, S // 2, TQ), U32),
            pltpu.VMEM((8, TQ), F32),
            pltpu.VMEM((1, TQ), F32),
            pltpu.VMEM((H, DH, TQ), F32),
            pltpu.VMEM((8, 128), U32),
            pltpu.VMEM((RV, 128), F32),
            pltpu.VMEM((1, DH, RV, 128), F32),
            pltpu.VMEM((2, DH + 8, TQ), F32),
            pltpu.VMEM((2, DH, TQ), U32),
            pltpu.VMEM((TQ, 128), BF16),
            pltpu.VMEM((TQ, D), F32),
            pltpu.VMEM((TQ, D), F32),
        ],
        compiler_params=pltpu.CompilerParams(
            dimension_semantics=("arbitrary",),
            vmem_limit_bytes=100 * 1024 * 1024,
        ),
    )(A_x, A_wq, A_wk.T, A_wv.T, A_wo, B_w1, B_w2)
```

```python
import math

import jax
import jax.numpy as jnp
import jax.experimental.pallas as pl
import jax.experimental.pallas.tpu as pltpu

F32 = jnp.float32
BF16 = jnp.bfloat16
U32 = jnp.uint32

S = 2048
D = 512
H = 32
DH = 16
FF = 1792
TQ = 512
NL = TQ // 128
NQ = S // TQ
NT = S // 128
NFC = FF // 128
EPS = 1e-5
KSCALE = (DH ** -0.5) * math.log2(math.e)
CH = 256
NCH = S // CH
NP = 4
HP = H // NP
L_SAFE = 2.0 ** -40
UP = 1.0 + 2.0 ** -6
TINY = 1e-30
W = 3
ND = 16

RJ = 2


class _Head:
    def __init__(self, rv):
        self.g0 = rv // 16
        g = (S - rv) // 16
        self.bounds = [g * c // ND for c in range(ND + 1)]
        self.vsteps = [(j, t) for j in range(NL) for t in range(rv // (16 * W))]
        self.nvt = -(-rv // 128)
        self.pv_order = list(range(self.nvt, NT)) + list(range(self.nvt))


class _Body:
    def __init__(self, pv, ffn, rvs, v0, tail, relt, rho, foff=None, lat=128):
        self.heads = [_Head(rv) for rv in rvs]
        self.pv = pv
        self.events = []
        slots = []
        fast = [(-lat, 0)]
        t = 0
        for u in range(len(pv)):
            for c in range(ND):
                if u < len(rvs):
                    for g in range(self.heads[u].bounds[c], self.heads[u].bounds[c + 1]):
                        slots.append(((u, g), t, len(self.events)))
                        t += 16
                self.events.append(("a", u, c))
                t += 16 if pv[u] else 0
                if ffn[u] and c == ND // 2 + foff[u]:
                    fast.append((t, t + TQ))
                    for g in range(TQ // 16):
                        slots.append(((u, "f", g), t, len(self.events)))
                        t += 16
                    self.events.append(("f", u, ffn[u]))
        tmax = slots[-1][1] + tail
        vt = [0.0]
        for x in range(tmax + 1):
            vt.append(vt[-1] + (rho if any(a <= x - lat < b for a, b in fast) else 1.0))
        ev = {e: m for m, e in enumerate(self.events)}
        self.steps = [(u, v) for u, hd in enumerate(self.heads) for v in range(len(hd.vsteps))]
        n = len(self.steps)
        self.dl, self.rel, self.at = [], [], []
        for k, (u, _) in enumerate(self.steps):
            latest = ev[("a", u + 1, NT - self.heads[u].nvt)] if u + 1 < len(pv) else len(self.events)
            want = vt[v0] + (vt[tmax] - vt[v0]) * k / (n - 1)
            td = min(x for x in range(tmax + 1) if vt[x] >= want - 1e-6)
            cand = [sl for sl in slots if sl[1] >= td and sl[0] not in self.dl]
            if cand:
                self.dl.append(cand[0][0])
                self.at.append(cand[0][2])
                td = cand[0][1]
            else:
                self.dl.append(None)
                self.at.append(latest)
            assert self.at[-1] <= latest
            assert u == 0 or self.at[-1] > ev[("a", u - 1, self.heads[u].nvt - 1)]
            cand = [sl for sl in slots if sl[1] <= td - relt]
            self.rel.append(cand[-1][0] if cand else None)


FIRST = _Body([False], [0], rvs=[288], v0=96, tail=128, relt=240, rho=1.0)
PBODY = _Body([True, True], [0, 0], rvs=[336, 288], v0=80, tail=128, relt=256, rho=1.1)
FBODY = _Body([True, True], [2, 1], rvs=[384, 384], foff=[7, -1], v0=112, tail=136, relt=256, rho=1.16,
              lat=144)
LAST = _Body([True, True], [2, 0], rvs=[384], foff=[5], v0=96, tail=128, relt=240, rho=1.2)
RV = max(hd.g0 * 16 for b in (FIRST, PBODY, FBODY, LAST) for hd in b.heads)
KB0 = -(-RV // CH)

NT_DIMS = (((1,), (1,)), ((), ()))


def _pk(x):
    return pltpu.bitcast(x, U32)


def _upk(x):
    return pltpu.bitcast(x, BF16)


def _layernorm(x, hook=None):
    x = x.astype(F32)
    mu = jnp.mean(x, axis=-1, keepdims=True)
    if hook is not None:
        mu = hook(mu)
    xc = x - mu
    var = jnp.mean(xc * xc, axis=-1, keepdims=True)
    return (xc * jax.lax.rsqrt(var + EPS)).astype(BF16)


def _kernel(x_hbm, wq_hbm, wkt_hbm, wvt_hbm, wo_hbm, w1_hbm, w2_hbm, o_ref,
            x_scr, wq_scr, wkt_scr, wvt_scr, wo_scr, w1_scr, w2_scr, sems,
            xn_scr, wt_scr, k_scr, vt_scr, kmax_scr, qt_scr, p_scr, l_scr, bad_scr, ot_scr,
            z_scr, kvo_scr, kb_scr, qc_scr, qtc_scr, h_scr, acc_scr, bak_scr):
    i = pl.program_id(0)

    def x_copy(c):
        rows = pl.ds(c * CH, CH)
        return pltpu.make_async_copy(x_hbm.at[0, rows, :], x_scr.at[rows, :], sems.at[c])

    wq_copy = pltpu.make_async_copy(wq_hbm, wq_scr, sems.at[NCH])
    kv_copies = [pltpu.make_async_copy(wkt_hbm, wkt_scr, sems.at[NCH + 4]),
                 pltpu.make_async_copy(wvt_hbm, wvt_scr, sems.at[NCH + 5])]
    w_copies = [pltpu.make_async_copy(w1_hbm, w1_scr, sems.at[NCH + 1]),
                pltpu.make_async_copy(w2_hbm, w2_scr, sems.at[NCH + 2]),
                pltpu.make_async_copy(wo_hbm, wo_scr, sems.at[NCH + 3])]

    def tie(x, dep):
        n = x.shape[0] // 8
        rep = lambda v: v if v.shape[0] == x.shape[0] else jnp.concatenate([v] * n, axis=0)
        z = z_scr[...] if dep.shape[0] == 8 else rep(z_scr[...])
        r = rep(pltpu.bitcast(dep, U32) & z)
        return pltpu.bitcast(pltpu.bitcast(x, U32) | r, x.dtype)

    def store_p(p, r0, nr, slot):
        p4 = p.reshape(nr // 16, 2, 8, TQ)
        pp = pltpu.pack_elementwise([p4[:, 0], p4[:, 1]], packed_dtype=BF16)
        p_scr[slot, r0 // 2:(r0 + nr) // 2, :] = pp.reshape(nr // 2, TQ).astype(U32)
        return jnp.sum(p.reshape(nr // 8, 8, TQ), axis=0)

    def qk_dot(hd, u, c, slot, l, deps, rels):
        g0, g1 = hd.bounds[c], hd.bounds[c + 1]
        ks = []
        for g in range(g0, g1):
            kv = k_scr[(hd.g0 + g) * 8:(hd.g0 + g + 1) * 8, :]
            if (u, g) in deps:
                kv = tie(kv, deps[(u, g)])
            ks.append(kv)
        kk = _upk(jnp.concatenate(ks, axis=0))[:, :2 * DH]
        s = jnp.dot(kk, _upk(qtc_scr[slot]), preferred_element_type=F32)
        for g in range(g0, g1):
            if (u, g) in rels:
                r0 = (g - g0) * 16
                rels[(u, g)] = s[r0:r0 + 8, RJ * 128:(RJ + 1) * 128]
        return l + store_p(jnp.exp2(s), (hd.g0 + g0) * 16, (g1 - g0) * 16, slot)

    def vpu_step(j, t, slot, lv, acc, rel):
        c0 = j * 128
        if t == 0:
            m8 = jnp.broadcast_to(qc_scr[slot, DH:DH + 1, c0:c0 + 128], (8, 128)) * kmax_scr[...]
            if rel is not None:
                m8 = tie(m8, rel)
            mm = jnp.concatenate([m8] * W, axis=0)
            acc = mm if acc is None else tie(mm, acc)
        elif rel is not None:
            acc = tie(acc, rel)
        ps = []
        for b in range(2):
            r0 = (2 * t + b) * 8 * W
            for d in range(DH):
                acc = acc + kb_scr[d, r0:r0 + 8 * W, :] * qc_scr[slot, d:d + 1, c0:c0 + 128]
            ps.append(jnp.exp2(acc))
        pp = pltpu.pack_elementwise(ps, packed_dtype=BF16)
        p_scr[slot, t * 8 * W:(t + 1) * 8 * W, c0:c0 + 128] = pp.astype(U32)
        return lv + jnp.sum((ps[0] + ps[1]).reshape(W, 8, 128), axis=0), acc

    def pv_tile(t, slot, acc):
        return acc + jnp.dot(_upk(vt_scr[:, t * 128:(t + 1) * 128]),
                             _upk(p_scr[slot, t * 64:(t + 1) * 64, :]),
                             preferred_element_type=F32)

    def finish(h, acc, l):
        lsum = jnp.sum(l, axis=0, keepdims=True)
        ot_scr[h] = acc / lsum
        return lsum

    def stage_q(n, slot):
        q = qt_scr[n]
        qtc_scr[slot] = q
        qc_scr[slot] = _upk(q).astype(F32)[:DH + 8]

    def stage_tile(t):
        acc_scr[...] = x_scr[pl.ds(pl.multiple_of(t * TQ, TQ), TQ), :].astype(F32)

    def ffn_dot(kind, u, f, deps, rels):
        if kind == 1:
            wrap = f + 1 >= NFC
            f = jnp.where(wrap, 0, f + 1)
            t = jnp.where(wrap, jnp.minimum(i + 1, NQ - 1), i)
            lhs = xn_scr[pl.ds(pl.multiple_of(t * (TQ // 2), TQ // 2), TQ // 2), :]
        else:
            lhs = _pk(h_scr[...])
        fcols = pl.ds(pl.multiple_of(f * 128, 128), 128)
        gs = []
        for g in range(TQ // 16):
            x = lhs[g * 8:(g + 1) * 8]
            if (u, "f", g) in deps:
                x0 = tie(x[:, :128], deps[(u, "f", g)])
                x = x0 if kind == 2 else jnp.concatenate([x0, x[:, 128:]], axis=1)
            gs.append(x)
        lhs = _upk(jnp.concatenate(gs, axis=0))
        r = jnp.dot(lhs, w1_scr[:, fcols] if kind == 1 else w2_scr[fcols, :], preferred_element_type=F32)
        for g in range(TQ // 16):
            if (u, "f", g) in rels:
                rels[(u, "f", g)] = r[g * 16:g * 16 + 8, :128]
        if kind == 1:
            a = 0.5 * r
            h_scr[...] = (a * jnp.tanh(a) + a).astype(BF16)
        else:
            acc_scr[...] += r

    def run_body(bd, slot0, h, f):
        nu, nh = len(bd.pv), len(bd.heads)
        l = [jnp.zeros((8, TQ), F32) for _ in range(nh)]
        lv = [[jnp.zeros((8, 128), F32) for _ in range(NL)] for _ in range(nh)]
        acc = [jnp.zeros((DH, TQ), F32) for _ in range(nu)]
        lprev = l_scr[...] if bd.pv[0] else None
        orders = [list(range(NT))] + [hd.pv_order for hd in bd.heads]
        ltot = lambda u: l[u] + jnp.concatenate(lv[u], axis=1)
        deps = {}
        rels = {key: None for key in bd.rel}
        vacc = None
        k = 0
        for m in range(len(bd.events) + 1):
            while k < len(bd.steps) and bd.at[k] <= m:
                u, v = bd.steps[k]
                j, t = bd.heads[u].vsteps[v]
                lv[u][j], vacc = vpu_step(j, t, (slot0 + u) % 2, lv[u][j], vacc, rels[bd.rel[k]])
                if bd.dl[k] is not None:
                    deps[bd.dl[k]] = lv[u][j]
                k += 1
            if m == len(bd.events):
                break
            kind, u, c = bd.events[m]
            if kind == "f":
                ffn_dot(c, u, f, deps, rels)
                continue
            if u < nh:
                l[u] = qk_dot(bd.heads[u], u, c, (slot0 + u) % 2, l[u], deps, rels)
            if bd.pv[u]:
                acc[u] = pv_tile(orders[u][c], (slot0 + u + 1) % 2, acc[u])
                if c == ND - 1 and u + 1 < nu:
                    lsum = finish(h + u, acc[u], lprev if u == 0 else ltot(u - 1))
                    bad_scr[...] = jnp.where(lsum >= L_SAFE, bad_scr[...], 1.0)
        if bd.pv[nu - 1]:
            lsum = finish(h + nu - 1, acc[nu - 1], lprev if nu == 1 else ltot(nu - 2))
            bad_scr[...] = jnp.where(lsum >= L_SAFE, bad_scr[...], 1.0)
        if nh == nu:
            l_scr[...] = ltot(nu - 1)

    def split_pairs(k):
        n = k.shape[0]
        kp = _pk(k.astype(BF16))
        ev = pltpu.bitcast(kp << 16, F32)
        od = pltpu.bitcast(kp & jnp.uint32(0xFFFF0000), F32)
        return ev.reshape(n // 16, 8, 128), od.reshape(n // 16, 8, 128)

    @pl.when(i == 0)
    def _():
        x_copy(0).start()
        for cp in kv_copies:
            cp.start()
        wq_copy.start()
        for c in range(1, NCH):
            x_copy(c).start()
        z_scr[...] = jnp.zeros((8, 128), U32)
        x_copy(0).wait()
        xn_scr[0:CH // 2, :] = _pk(_layernorm(x_scr[0:CH, :]))
        for cp in kv_copies:
            cp.wait()
        wq_copy.wait()
        x_copy(1).wait()
        x_copy(2).wait()
        wkv = jnp.concatenate([wkt_scr[...].astype(F32), wvt_scr[...].astype(F32)], axis=0)
        wt_scr[:DH, :] = _pk(wkv.astype(BF16))
        wt_scr[DH:, :] = _pk(wq_scr[...].astype(F32).T.astype(BF16))

        row = jax.lax.broadcasted_iota(jnp.int32, (HP, 8, CH), 1)
        kmax2 = jnp.zeros((1, CH), F32)
        evs, ods = [], []
        prev_res = None
        nslots = (NCH - KB0) * NP
        for c in range(NCH):
            if c == 2:
                prev_res = None
                for cw in range(3, NCH):
                    x_copy(cw).wait()
                for cp in w_copies:
                    cp.start()
            half = pl.ds(c * (CH // 2), CH // 2)
            xn = _upk(xn_scr[half, :])
            tile = c // (TQ // CH)
            cols = pl.ds((c % (TQ // CH)) * CH, CH)
            for pc in range(NP):
                if c < NCH - 1:
                    qr = CH // NP
                    q0 = (c + 1) * CH + pc * qr
                    hook = None
                    if prev_res is not None:
                        def hook(mu, dep=prev_res):
                            return tie(jnp.broadcast_to(mu, (qr, 128)), dep)[:, :1]
                    xn_scr[q0 // 2:(q0 + qr) // 2, :] = _pk(_layernorm(x_scr[q0:q0 + qr, :], hook))
                r1 = 2 * DH + (pc + 1) * HP * DH
                r0 = 0 if pc == 0 else r1 - HP * DH
                t_all = jax.lax.dot_general(_upk(wt_scr[r0 // 2:r1 // 2, :]), xn, NT_DIMS,
                                            preferred_element_type=F32)
                if pc == 0:
                    vt_scr[:, pl.ds(c * CH, CH)] = _pk(t_all[DH:2 * DH].astype(BF16))
                    kt = (t_all[:DH] * KSCALE).astype(BF16).astype(F32)
                    kmax2 = jnp.maximum(kmax2, jnp.sum(kt * kt, axis=0, keepdims=True))
                    k = jnp.concatenate([kt, jnp.zeros((128 - DH, CH), F32)], axis=0).T
                    ev, od = split_pairs(k)
                    kperm = jnp.concatenate([ev[:, None], od[:, None]], axis=1).reshape(CH, 128)
                    k_scr[half, :] = _pk(kperm.astype(BF16))
                    if c < KB0:
                        evs.append(ev)
                        ods.append(od)
                    if c == KB0 - 1:
                        ev = jnp.concatenate(evs, axis=0)
                        od = jnp.concatenate(ods, axis=0)
                        parts = []
                        for t in range(RV // (16 * W)):
                            parts.append(ev[W * t:W * (t + 1)].reshape(8 * W, 128))
                            parts.append(od[W * t:W * (t + 1)].reshape(8 * W, 128))
                        kvo = jnp.concatenate(parts, axis=0)
                        kvo_scr[...] = jnp.concatenate(
                            [kvo[:8 * W], kvo[8 * W:] - kvo[:RV - 8 * W]], axis=0)
                    t_all = t_all[2 * DH:]
                prev_res = t_all[0:8, 0:128]
                q3 = t_all.reshape(HP, DH, CH)
                q2 = jnp.sum(q3 * q3, axis=1, keepdims=True) + TINY
                qn = q2 * jax.lax.rsqrt(q2) * (-UP)
                qnw = pltpu.bitcast(jnp.broadcast_to(qn, (HP, 8, CH)), U32) >> 16
                qp = jnp.concatenate([_pk(t_all.astype(BF16)).reshape(HP, 8, CH),
                                      jnp.where(row == 0, qnw, jnp.uint32(0))], axis=1)
                qt_scr[pl.ds(tile * H + pc * HP, HP), :, cols] = qp
                if c >= KB0:
                    sl = (c - KB0) * NP + pc
                    for d in range(DH * sl // nslots, DH * (sl + 1) // nslots):
                        src = tie(kvo_scr[...], t_all[0:8, 0:128])
                        kb_scr[d] = jnp.broadcast_to(src[:, d:d + 1], (RV, 128))

        km2 = jnp.broadcast_to(jnp.max(kmax2, axis=1, keepdims=True), (8, 128))
        km = (jnp.sqrt(km2) * UP).astype(BF16).astype(F32)
        kmax_scr[...] = km
        kmw = _pk(jnp.concatenate([km, km], axis=0).astype(BF16))
        lane = jax.lax.broadcasted_iota(jnp.int32, (S // 16, 8, 128), 2)
        k_scr[...] = jnp.where(lane == DH, kmw[None], k_scr[...].reshape(S // 16, 8, 128)).reshape(S // 2, 128)
        stage_tile(0)
        stage_q(0, 0)
        stage_q(1, 1)
        run_body(FIRST, 0, None, None)
        stage_q(2, 0)

    bad_scr[...] = jnp.zeros((1, TQ), F32)
    n0 = i * H
    last = NQ * H - 1

    def pbody(hh, carry):
        h = 2 * hh
        run_body(PBODY, 1, h, None)
        stage_q(n0 + h + 3, 1)
        stage_q(n0 + h + 4, 0)
        return carry

    jax.lax.fori_loop(0, H // 2 - NFC, pbody, 0)

    @pl.when(i == 0)
    def _():
        for cp in w_copies:
            cp.wait()
        ffn_dot(1, 0, -1, {}, {})

    def fbody(hh, carry):
        h = H - 2 * NFC + 2 * hh
        run_body(FBODY, 1, h, hh)
        stage_q(jnp.minimum(n0 + h + 3, last), 1)
        stage_q(jnp.minimum(n0 + h + 4, last), 0)
        return carry

    is_last = i == NQ - 1
    jax.lax.fori_loop(0, NFC - is_last.astype(jnp.int32), fbody, 0)

    @pl.when(is_last)
    def _():
        run_body(LAST, 1, H - 2, NFC - 1)

    def out_proj(base):
        o = ot_scr[...].reshape(D, TQ).T.astype(BF16)
        o_ref[0] = (jnp.dot(o, wo_scr[...], preferred_element_type=F32) + base).astype(BF16)

    unsafe = jnp.max(bad_scr[...]) > 0.0
    base = acc_scr[...]
    bak_scr[...] = base
    out_proj(base)
    stage_tile(jnp.minimum(i + 1, NQ - 1))

    @pl.when(unsafe)
    def _():
        def slow_head(h, carry):
            kk = _upk(k_scr[...])[:, :DH]
            s = jnp.dot(kk, _upk(qt_scr[n0 + h, 0:DH // 2, :]), preferred_element_type=F32)
            m = jnp.max(s, axis=0, keepdims=True)
            l = store_p(jnp.exp2(s - m), 0, S, 1)
            acc = jnp.dot(_upk(vt_scr[...]), _upk(p_scr[1]), preferred_element_type=F32)
            finish(h, acc, l)
            return carry

        jax.lax.fori_loop(0, H, slow_head, 0)
        out_proj(bak_scr[...])


@jax.jit
def pallas_parallel_sum__grouped_kv_mqa__dense_activation_silu__prompt_kernel(
    A_x: jax.Array,
    A_wq: jax.Array,
    A_wk: jax.Array,
    A_wv: jax.Array,
    A_wo: jax.Array,
    B_x: jax.Array,
    B_w1: jax.Array,
    B_w2: jax.Array,
):
    del B_x
    hbm = pl.BlockSpec(memory_space=pl.ANY)
    return pl.pallas_call(
        _kernel,
        out_shape=jax.ShapeDtypeStruct((1, S, D), BF16),
        grid=(NQ,),
        in_specs=[hbm] * 7,
        out_specs=pl.BlockSpec((1, TQ, D), lambda i: (0, i, 0)),
        scratch_shapes=[
            pltpu.VMEM((S, D), BF16),
            pltpu.VMEM((D, D), BF16),
            pltpu.VMEM((DH, D), BF16),
            pltpu.VMEM((DH, D), BF16),
            pltpu.VMEM((D, D), BF16),
            pltpu.VMEM((D, FF), BF16),
            pltpu.VMEM((FF, D), BF16),
            pltpu.SemaphoreType.DMA((NCH + 6,)),
            pltpu.VMEM((S // 2, D), U32),
            pltpu.VMEM((D // 2 + DH, D), U32),
            pltpu.VMEM((S // 2, 128), U32),
            pltpu.VMEM((DH // 2, S), U32),
            pltpu.VMEM((8, 128), F32),
            pltpu.VMEM((NQ * H, DH, TQ), U32),
            pltpu.VMEM((2, S // 2, TQ), U32),
            pltpu.VMEM((8, TQ), F32),
            pltpu.VMEM((1, TQ), F32),
            pltpu.VMEM((H, DH, TQ), F32),
            pltpu.VMEM((8, 128), U32),
            pltpu.VMEM((RV, 128), F32),
            pltpu.VMEM((DH, RV, 128), F32),
            pltpu.VMEM((2, DH + 8, TQ), F32),
            pltpu.VMEM((2, DH, TQ), U32),
            pltpu.VMEM((TQ, 128), BF16),
            pltpu.VMEM((TQ, D), F32),
            pltpu.VMEM((TQ, D), F32),
        ],
        compiler_params=pltpu.CompilerParams(
            dimension_semantics=("arbitrary",),
            vmem_limit_bytes=100 * 1024 * 1024,
        ),
    )(A_x, A_wq, A_wk.T, A_wv.T, A_wo, B_w1, B_w2)
```

```python
import math

import jax
import jax.numpy as jnp
import jax.experimental.pallas as pl
import jax.experimental.pallas.tpu as pltpu

F32 = jnp.float32
BF16 = jnp.bfloat16
U32 = jnp.uint32

S = 2048
D = 512
H = 32
DH = 16
FF = 1792
TQ = 512
NL = TQ // 128
NQ = S // TQ
NT = S // 128
NFC = FF // 128
EPS = 1e-5
KSCALE = (DH ** -0.5) * math.log2(math.e)
CH = 256
NCH = S // CH
NP = 4
HP = H // NP
L_SAFE = 2.0 ** -40
UP = 1.0 + 2.0 ** -6
TINY = 1e-30
W = 3
ND = 16

RJ = 2


class _Head:
    def __init__(self, rv):
        self.g0 = rv // 16
        g = (S - rv) // 16
        self.bounds = [g * c // ND for c in range(ND + 1)]
        self.vsteps = [(j, t) for j in range(NL) for t in range(rv // (16 * W))]
        self.nvt = -(-rv // 128)
        self.pv_order = list(range(self.nvt, NT)) + list(range(self.nvt))


class _Body:
    def __init__(self, pv, ffn, rvs, v0, tail, relt, rho, foff=None, lat=128):
        self.heads = [_Head(rv) for rv in rvs]
        self.pv = pv
        self.events = []
        slots = []
        fast = [(-lat, 0)]
        t = 0
        for u in range(len(pv)):
            for c in range(ND):
                if u < len(rvs):
                    for g in range(self.heads[u].bounds[c], self.heads[u].bounds[c + 1]):
                        slots.append(((u, g), t, len(self.events)))
                        t += 16
                self.events.append(("a", u, c))
                t += 16 if pv[u] else 0
                if ffn[u] and c == ND // 2 + foff[u]:
                    fast.append((t, t + TQ))
                    for g in range(TQ // 16):
                        slots.append(((u, "f", g), t, len(self.events)))
                        t += 16
                    self.events.append(("f", u, ffn[u]))
        tmax = slots[-1][1] + tail
        vt = [0.0]
        for x in range(tmax + 1):
            vt.append(vt[-1] + (rho if any(a <= x - lat < b for a, b in fast) else 1.0))
        ev = {e: m for m, e in enumerate(self.events)}
        self.steps = [(u, v) for u, hd in enumerate(self.heads) for v in range(len(hd.vsteps))]
        n = len(self.steps)
        self.dl, self.rel, self.at = [], [], []
        for k, (u, _) in enumerate(self.steps):
            latest = ev[("a", u + 1, NT - self.heads[u].nvt)] if u + 1 < len(pv) else len(self.events)
            want = vt[v0] + (vt[tmax] - vt[v0]) * k / (n - 1)
            td = min(x for x in range(tmax + 1) if vt[x] >= want - 1e-6)
            cand = [sl for sl in slots if sl[1] >= td and sl[0] not in self.dl]
            if cand:
                self.dl.append(cand[0][0])
                self.at.append(cand[0][2])
                td = cand[0][1]
            else:
                self.dl.append(None)
                self.at.append(latest)
            assert self.at[-1] <= latest
            assert u == 0 or self.at[-1] > ev[("a", u - 1, self.heads[u].nvt - 1)]
            cand = [sl for sl in slots if sl[1] <= td - relt]
            self.rel.append(cand[-1][0] if cand else None)


FIRST = _Body([False], [0], rvs=[288], v0=96, tail=128, relt=240, rho=1.0)
PBODY = _Body([True, True], [0, 0], rvs=[336, 288], v0=80, tail=128, relt=256, rho=1.1)
FBODY = _Body([True, True], [2, 1], rvs=[384, 384], foff=[7, -1], v0=112, tail=136, relt=256, rho=1.16,
              lat=144)
LAST = _Body([True, True], [2, 0], rvs=[384], foff=[5], v0=96, tail=128, relt=240, rho=1.2)
RV = max(hd.g0 * 16 for b in (FIRST, PBODY, FBODY, LAST) for hd in b.heads)
KB0 = -(-RV // CH)

NT_DIMS = (((1,), (1,)), ((), ()))


def _pk(x):
    return pltpu.bitcast(x, U32)


def _upk(x):
    return pltpu.bitcast(x, BF16)


def _layernorm(x, hook=None):
    x = x.astype(F32)
    mu = jnp.mean(x, axis=-1, keepdims=True)
    if hook is not None:
        mu = hook(mu)
    xc = x - mu
    var = jnp.mean(xc * xc, axis=-1, keepdims=True)
    return (xc * jax.lax.rsqrt(var + EPS)).astype(BF16)


def _kernel(x_hbm, wq_hbm, wkt_hbm, wvt_hbm, wo_hbm, w1_hbm, w2_hbm, o_ref,
            x_scr, wq_scr, wkt_scr, wvt_scr, wo_scr, w1_scr, w2_scr, sems,
            xn_scr, wt_scr, k_scr, vt_scr, kmax_scr, qt_scr, p_scr, l_scr, bad_scr, ot_scr,
            z_scr, kvo_scr, kb_scr, qc_scr, qtc_scr, h_scr, acc_scr, bak_scr):
    i = pl.program_id(0)

    def x_copy(c):
        rows = pl.ds(c * CH, CH)
        return pltpu.make_async_copy(x_hbm.at[0, rows, :], x_scr.at[rows, :], sems.at[c])

    wq_copy = pltpu.make_async_copy(wq_hbm, wq_scr, sems.at[NCH])
    kv_copies = [pltpu.make_async_copy(wkt_hbm, wkt_scr, sems.at[NCH + 4]),
                 pltpu.make_async_copy(wvt_hbm, wvt_scr, sems.at[NCH + 5])]
    w_copies = [pltpu.make_async_copy(w1_hbm, w1_scr, sems.at[NCH + 1]),
                pltpu.make_async_copy(w2_hbm, w2_scr, sems.at[NCH + 2]),
                pltpu.make_async_copy(wo_hbm, wo_scr, sems.at[NCH + 3])]

    def tie(x, dep):
        n = x.shape[0] // 8
        rep = lambda v: v if v.shape[0] == x.shape[0] else jnp.concatenate([v] * n, axis=0)
        z = z_scr[...] if dep.shape[0] == 8 else rep(z_scr[...])
        r = rep(pltpu.bitcast(dep, U32) & z)
        return pltpu.bitcast(pltpu.bitcast(x, U32) | r, x.dtype)

    def store_p(p, r0, nr, slot):
        p4 = p.reshape(nr // 16, 2, 8, TQ)
        pp = pltpu.pack_elementwise([p4[:, 0], p4[:, 1]], packed_dtype=BF16)
        p_scr[slot, r0 // 2:(r0 + nr) // 2, :] = pp.reshape(nr // 2, TQ).astype(U32)
        return jnp.sum(p.reshape(nr // 8, 8, TQ), axis=0)

    def qk_dot(hd, u, c, slot, l, deps, rels):
        g0, g1 = hd.bounds[c], hd.bounds[c + 1]
        ks = []
        for g in range(g0, g1):
            kv = k_scr[(hd.g0 + g) * 8:(hd.g0 + g + 1) * 8, :]
            if (u, g) in deps:
                kv = tie(kv, deps[(u, g)])
            ks.append(kv)
        kk = _upk(jnp.concatenate(ks, axis=0))[:, :2 * DH]
        s = jnp.dot(kk, _upk(qtc_scr[slot]), preferred_element_type=F32)
        for g in range(g0, g1):
            if (u, g) in rels:
                r0 = (g - g0) * 16
                rels[(u, g)] = s[r0:r0 + 8, RJ * 128:(RJ + 1) * 128]
        return l + store_p(jnp.exp2(s), (hd.g0 + g0) * 16, (g1 - g0) * 16, slot)

    def vpu_step(j, t, slot, lv, acc, rel):
        c0 = j * 128
        if t == 0:
            m8 = jnp.broadcast_to(qc_scr[slot, DH:DH + 1, c0:c0 + 128], (8, 128)) * kmax_scr[...]
            if rel is not None:
                m8 = tie(m8, rel)
            mm = jnp.concatenate([m8] * W, axis=0)
            acc = mm if acc is None else tie(mm, acc)
        elif rel is not None:
            acc = tie(acc, rel)
        ps = []
        qb = {}
        for b in range(2):
            r0 = (2 * t + b) * 8 * W
            for d in range(DH):
                kb = kb_scr[d, r0:r0 + 8 * W, :]
                if b == 0:
                    qb[d] = qc_scr[slot, d:d + 1, c0:c0 + 128]
                acc = acc + kb * qb[d]
            ps.append(jnp.exp2(acc))
        pp = pltpu.pack_elementwise(ps, packed_dtype=BF16)
        p_scr[slot, t * 8 * W:(t + 1) * 8 * W, c0:c0 + 128] = pp.astype(U32)
        return lv + jnp.sum((ps[0] + ps[1]).reshape(W, 8, 128), axis=0), acc

    def pv_tile(t, slot, acc):
        return acc + jnp.dot(_upk(vt_scr[:, t * 128:(t + 1) * 128]),
                             _upk(p_scr[slot, t * 64:(t + 1) * 64, :]),
                             preferred_element_type=F32)

    def finish(h, acc, l):
        lsum = jnp.sum(l, axis=0, keepdims=True)
        ot_scr[h] = acc / lsum
        return lsum

    def stage_q(n, slot):
        q = qt_scr[n]
        qtc_scr[slot] = q
        qc_scr[slot] = _upk(q).astype(F32)[:DH + 8]

    def stage_tile(t):
        acc_scr[...] = x_scr[pl.ds(pl.multiple_of(t * TQ, TQ), TQ), :].astype(F32)

    def ffn_dot(kind, u, f, deps, rels):
        if kind == 1:
            wrap = f + 1 >= NFC
            f = jnp.where(wrap, 0, f + 1)
            t = jnp.where(wrap, jnp.minimum(i + 1, NQ - 1), i)
            lhs = xn_scr[pl.ds(pl.multiple_of(t * (TQ // 2), TQ // 2), TQ // 2), :]
        else:
            lhs = _pk(h_scr[...])
        fcols = pl.ds(pl.multiple_of(f * 128, 128), 128)
        gs = []
        for g in range(TQ // 16):
            x = lhs[g * 8:(g + 1) * 8]
            if (u, "f", g) in deps:
                x0 = tie(x[:, :128], deps[(u, "f", g)])
                x = x0 if kind == 2 else jnp.concatenate([x0, x[:, 128:]], axis=1)
            gs.append(x)
        lhs = _upk(jnp.concatenate(gs, axis=0))
        r = jnp.dot(lhs, w1_scr[:, fcols] if kind == 1 else w2_scr[fcols, :], preferred_element_type=F32)
        for g in range(TQ // 16):
            if (u, "f", g) in rels:
                rels[(u, "f", g)] = r[g * 16:g * 16 + 8, :128]
        if kind == 1:
            a = 0.5 * r
            h_scr[...] = (a * jnp.tanh(a) + a).astype(BF16)
        else:
            acc_scr[...] += r

    def run_body(bd, slot0, h, f):
        nu, nh = len(bd.pv), len(bd.heads)
        l = [jnp.zeros((8, TQ), F32) for _ in range(nh)]
        lv = [[jnp.zeros((8, 128), F32) for _ in range(NL)] for _ in range(nh)]
        acc = [jnp.zeros((DH, TQ), F32) for _ in range(nu)]
        lprev = l_scr[...] if bd.pv[0] else None
        orders = [list(range(NT))] + [hd.pv_order for hd in bd.heads]
        ltot = lambda u: l[u] + jnp.concatenate(lv[u], axis=1)
        deps = {}
        rels = {key: None for key in bd.rel}
        vacc = None
        k = 0
        for m in range(len(bd.events) + 1):
            while k < len(bd.steps) and bd.at[k] <= m:
                u, v = bd.steps[k]
                j, t = bd.heads[u].vsteps[v]
                lv[u][j], vacc = vpu_step(j, t, (slot0 + u) % 2, lv[u][j], vacc, rels[bd.rel[k]])
                if bd.dl[k] is not None:
                    deps[bd.dl[k]] = lv[u][j]
                k += 1
            if m == len(bd.events):
                break
            kind, u, c = bd.events[m]
            if kind == "f":
                ffn_dot(c, u, f, deps, rels)
                continue
            if u < nh:
                l[u] = qk_dot(bd.heads[u], u, c, (slot0 + u) % 2, l[u], deps, rels)
            if bd.pv[u]:
                acc[u] = pv_tile(orders[u][c], (slot0 + u + 1) % 2, acc[u])
                if c == ND - 1 and u + 1 < nu:
                    lsum = finish(h + u, acc[u], lprev if u == 0 else ltot(u - 1))
                    bad_scr[...] = jnp.where(lsum >= L_SAFE, bad_scr[...], 1.0)
        if bd.pv[nu - 1]:
            lsum = finish(h + nu - 1, acc[nu - 1], lprev if nu == 1 else ltot(nu - 2))
            bad_scr[...] = jnp.where(lsum >= L_SAFE, bad_scr[...], 1.0)
        if nh == nu:
            l_scr[...] = ltot(nu - 1)

    def split_pairs(k):
        n = k.shape[0]
        kp = _pk(k.astype(BF16))
        ev = pltpu.bitcast(kp << 16, F32)
        od = pltpu.bitcast(kp & jnp.uint32(0xFFFF0000), F32)
        return ev.reshape(n // 16, 8, 128), od.reshape(n // 16, 8, 128)

    @pl.when(i == 0)
    def _():
        x_copy(0).start()
        for cp in kv_copies:
            cp.start()
        wq_copy.start()
        for c in range(1, NCH):
            x_copy(c).start()
        z_scr[...] = jnp.zeros((8, 128), U32)
        x_copy(0).wait()
        xn_scr[0:CH // 2, :] = _pk(_layernorm(x_scr[0:CH, :]))
        for cp in kv_copies:
            cp.wait()
        wq_copy.wait()
        x_copy(1).wait()
        x_copy(2).wait()
        wkv = jnp.concatenate([wkt_scr[...].astype(F32), wvt_scr[...].astype(F32)], axis=0)
        wt_scr[:DH, :] = _pk(wkv.astype(BF16))
        wt_scr[DH:, :] = _pk(wq_scr[...].astype(F32).T.astype(BF16))

        row = jax.lax.broadcasted_iota(jnp.int32, (HP, 8, CH), 1)
        kmax2 = jnp.zeros((1, CH), F32)
        evs, ods = [], []
        prev_res = None
        nslots = (NCH - KB0) * NP
        for c in range(NCH):
            if c == 2:
                prev_res = None
                for cw in range(3, NCH):
                    x_copy(cw).wait()
                for cp in w_copies:
                    cp.start()
            half = pl.ds(c * (CH // 2), CH // 2)
            xn = _upk(xn_scr[half, :])
            tile = c // (TQ // CH)
            cols = pl.ds((c % (TQ // CH)) * CH, CH)
            for pc in range(NP):
                if c < NCH - 1:
                    qr = CH // NP
                    q0 = (c + 1) * CH + pc * qr
                    hook = None
                    if prev_res is not None:
                        def hook(mu, dep=prev_res):
                            return tie(jnp.broadcast_to(mu, (qr, 128)), dep)[:, :1]
                    xn_scr[q0 // 2:(q0 + qr) // 2, :] = _pk(_layernorm(x_scr[q0:q0 + qr, :], hook))
                r1 = 2 * DH + (pc + 1) * HP * DH
                r0 = 0 if pc == 0 else r1 - HP * DH
                t_all = jax.lax.dot_general(_upk(wt_scr[r0 // 2:r1 // 2, :]), xn, NT_DIMS,
                                            preferred_element_type=F32)
                if pc == 0:
                    vt_scr[:, pl.ds(c * CH, CH)] = _pk(t_all[DH:2 * DH].astype(BF16))
                    kt = (t_all[:DH] * KSCALE).astype(BF16).astype(F32)
                    kmax2 = jnp.maximum(kmax2, jnp.sum(kt * kt, axis=0, keepdims=True))
                    k = jnp.concatenate([kt, jnp.zeros((128 - DH, CH), F32)], axis=0).T
                    ev, od = split_pairs(k)
                    kperm = jnp.concatenate([ev[:, None], od[:, None]], axis=1).reshape(CH, 128)
                    k_scr[half, :] = _pk(kperm.astype(BF16))
                    if c < KB0:
                        evs.append(ev)
                        ods.append(od)
                    if c == KB0 - 1:
                        ev = jnp.concatenate(evs, axis=0)
                        od = jnp.concatenate(ods, axis=0)
                        parts = []
                        for t in range(RV // (16 * W)):
                            parts.append(ev[W * t:W * (t + 1)].reshape(8 * W, 128))
                            parts.append(od[W * t:W * (t + 1)].reshape(8 * W, 128))
                        kvo = jnp.concatenate(parts, axis=0)
                        kvo_scr[...] = jnp.concatenate(
                            [kvo[:8 * W], kvo[8 * W:] - kvo[:RV - 8 * W]], axis=0)
                    t_all = t_all[2 * DH:]
                prev_res = t_all[0:8, 0:128]
                q3 = t_all.reshape(HP, DH, CH)
                q2 = jnp.sum(q3 * q3, axis=1, keepdims=True) + TINY
                qn = q2 * jax.lax.rsqrt(q2) * (-UP)
                qnw = pltpu.bitcast(jnp.broadcast_to(qn, (HP, 8, CH)), U32) >> 16
                qp = jnp.concatenate([_pk(t_all.astype(BF16)).reshape(HP, 8, CH),
                                      jnp.where(row == 0, qnw, jnp.uint32(0))], axis=1)
                qt_scr[pl.ds(tile * H + pc * HP, HP), :, cols] = qp
                if c >= KB0:
                    sl = (c - KB0) * NP + pc
                    for d in range(DH * sl // nslots, DH * (sl + 1) // nslots):
                        src = tie(kvo_scr[...], t_all[0:8, 0:128])
                        kb_scr[d] = jnp.broadcast_to(src[:, d:d + 1], (RV, 128))

        km2 = jnp.broadcast_to(jnp.max(kmax2, axis=1, keepdims=True), (8, 128))
        km = (jnp.sqrt(km2) * UP).astype(BF16).astype(F32)
        kmax_scr[...] = km
        kmw = _pk(jnp.concatenate([km, km], axis=0).astype(BF16))
        lane = jax.lax.broadcasted_iota(jnp.int32, (S // 16, 8, 128), 2)
        k_scr[...] = jnp.where(lane == DH, kmw[None], k_scr[...].reshape(S // 16, 8, 128)).reshape(S // 2, 128)
        stage_tile(0)
        stage_q(0, 0)
        stage_q(1, 1)
        run_body(FIRST, 0, None, None)
        stage_q(2, 0)

    bad_scr[...] = jnp.zeros((1, TQ), F32)
    n0 = i * H
    last = NQ * H - 1

    def pbody(hh, carry):
        h = 2 * hh
        run_body(PBODY, 1, h, None)
        stage_q(n0 + h + 3, 1)
        stage_q(n0 + h + 4, 0)
        return carry

    jax.lax.fori_loop(0, H // 2 - NFC, pbody, 0)

    @pl.when(i == 0)
    def _():
        for cp in w_copies:
            cp.wait()
        ffn_dot(1, 0, -1, {}, {})

    def fbody(hh, carry):
        h = H - 2 * NFC + 2 * hh
        run_body(FBODY, 1, h, hh)
        stage_q(jnp.minimum(n0 + h + 3, last), 1)
        stage_q(jnp.minimum(n0 + h + 4, last), 0)
        return carry

    is_last = i == NQ - 1
    jax.lax.fori_loop(0, NFC - is_last.astype(jnp.int32), fbody, 0)

    @pl.when(is_last)
    def _():
        run_body(LAST, 1, H - 2, NFC - 1)

    def out_proj(base):
        o = ot_scr[...].reshape(D, TQ).T.astype(BF16)
        o_ref[0] = (jnp.dot(o, wo_scr[...], preferred_element_type=F32) + base).astype(BF16)

    unsafe = jnp.max(bad_scr[...]) > 0.0
    base = acc_scr[...]
    bak_scr[...] = base
    out_proj(base)
    stage_tile(jnp.minimum(i + 1, NQ - 1))

    @pl.when(unsafe)
    def _():
        def slow_head(h, carry):
            kk = _upk(k_scr[...])[:, :DH]
            s = jnp.dot(kk, _upk(qt_scr[n0 + h, 0:DH // 2, :]), preferred_element_type=F32)
            m = jnp.max(s, axis=0, keepdims=True)
            l = store_p(jnp.exp2(s - m), 0, S, 1)
            acc = jnp.dot(_upk(vt_scr[...]), _upk(p_scr[1]), preferred_element_type=F32)
            finish(h, acc, l)
            return carry

        jax.lax.fori_loop(0, H, slow_head, 0)
        out_proj(bak_scr[...])


@jax.jit
def pallas_parallel_sum__grouped_kv_mqa__dense_activation_silu__prompt_kernel(
    A_x: jax.Array,
    A_wq: jax.Array,
    A_wk: jax.Array,
    A_wv: jax.Array,
    A_wo: jax.Array,
    B_x: jax.Array,
    B_w1: jax.Array,
    B_w2: jax.Array,
):
    del B_x
    hbm = pl.BlockSpec(memory_space=pl.ANY)
    return pl.pallas_call(
        _kernel,
        out_shape=jax.ShapeDtypeStruct((1, S, D), BF16),
        grid=(NQ,),
        in_specs=[hbm] * 7,
        out_specs=pl.BlockSpec((1, TQ, D), lambda i: (0, i, 0)),
        scratch_shapes=[
            pltpu.VMEM((S, D), BF16),
            pltpu.VMEM((D, D), BF16),
            pltpu.VMEM((DH, D), BF16),
            pltpu.VMEM((DH, D), BF16),
            pltpu.VMEM((D, D), BF16),
            pltpu.VMEM((D, FF), BF16),
            pltpu.VMEM((FF, D), BF16),
            pltpu.SemaphoreType.DMA((NCH + 6,)),
            pltpu.VMEM((S // 2, D), U32),
            pltpu.VMEM((D // 2 + DH, D), U32),
            pltpu.VMEM((S // 2, 128), U32),
            pltpu.VMEM((DH // 2, S), U32),
            pltpu.VMEM((8, 128), F32),
            pltpu.VMEM((NQ * H, DH, TQ), U32),
            pltpu.VMEM((2, S // 2, TQ), U32),
            pltpu.VMEM((8, TQ), F32),
            pltpu.VMEM((1, TQ), F32),
            pltpu.VMEM((H, DH, TQ), F32),
            pltpu.VMEM((8, 128), U32),
            pltpu.VMEM((RV, 128), F32),
            pltpu.VMEM((DH, RV, 128), F32),
            pltpu.VMEM((2, DH + 8, TQ), F32),
            pltpu.VMEM((2, DH, TQ), U32),
            pltpu.VMEM((TQ, 128), BF16),
            pltpu.VMEM((TQ, D), F32),
            pltpu.VMEM((TQ, D), F32),
        ],
        compiler_params=pltpu.CompilerParams(
            dimension_semantics=("arbitrary",),
            vmem_limit_bytes=100 * 1024 * 1024,
        ),
    )(A_x, A_wq, A_wk.T, A_wv.T, A_wo, B_w1, B_w2)
```
